```python
import jax
import jax.numpy as jnp

def _softmax(x, axis=-1):
    return jax.nn.softmax(x, axis=axis)
def _gelu(x):
    return jax.nn.gelu(x, approximate=True)
def _silu(x):
    return jax.nn.silu(x)
def _sigmoid(x):
    return jax.nn.sigmoid(x)
def _layernorm(x, axis=-1, eps=1e-5):
    m = jnp.mean(x, axis=axis, keepdims=True)
    v = jnp.var(x, axis=axis, keepdims=True)
    return (x - m) / jnp.sqrt(v + eps)
def _scatter_add(tgt, idx, src, axis=0):
    return tgt.at[idx].add(src)
def _segment_sum(src, seg, n):
    return jax.ops.segment_sum(src, seg, n)
class _Rng:
    def __init__(self, key):
        self._k = key
    def _next(self):
        self._k, sub = jax.random.split(self._k)
        return sub
    def normal(self, shape):
        return jax.random.normal(self._next(), shape, dtype=jnp.bfloat16)
    def randint(self, lo, hi, shape):
        return jax.random.randint(self._next(), shape, lo, hi, dtype=jnp.int32)
    def uniform(self, shape, lo=0.0, hi=1.0):
        return jax.random.uniform(self._next(), shape, jnp.bfloat16, lo, hi)
    def permutation(self, n):
        return jax.random.permutation(self._next(), n)


kernel_name = 'parallel_sum__sliding_block_cached__moe_arch_mod__decode'

def setup_inputs():
    _rng = _Rng(jax.random.key(int.from_bytes(__import__("os").urandom(4), "little")))
    _w = (lambda a: (lambda t: t.astype(jnp.bfloat16) if jnp.issubdtype(t.dtype, jnp.floating) else t)(jnp.asarray(a)))
    def _A_setup():
        B, Sq, D = 1, 1, 512
        Hq, Hkv, Sk, Dh = 32, 8, 65536, 128
        assert Hq % Hkv == 0, (Hq, Hkv)
        return {
            "x": _w((lambda *s: _rng.normal(s) * 0.05)(B, Sq, D)),
            "k_cache": _w((lambda *s: _rng.normal(s) * 0.05)(B, Hkv, Sk, Dh)),
            "v_cache": _w((lambda *s: _rng.normal(s) * 0.05)(B, Hkv, Sk, Dh)),
            "wq": _w((lambda *s: _rng.normal(s) * 0.05)(D, Hq * Dh) * (D ** -0.5)),
            "wo": _w((lambda *s: _rng.normal(s) * 0.05)(Hq * Dh, D) * ((Hq * Dh) ** -0.5)),
        }
    _A_in = _A_setup()

    def _B_setup():
        B, S, D, F, C = 1, 1, 512, 1792, 1
        return {
            "x": _w((lambda *s: _rng.normal(s) * 0.05)(B, S, D)),
            "w_r": _w((lambda *s: _rng.normal(s) * 0.05)(D)),
            "w_gate": _w((lambda *s: _rng.normal(s) * 0.05)(D, F)),
            "w_up": _w((lambda *s: _rng.normal(s) * 0.05)(D, F)),
            "w_down": _w((lambda *s: _rng.normal(s) * 0.05)(F, D)),
        }
    _B_in = _B_setup()

    return {
        "A_x": _A_in["x"],
        "A_k_cache": _A_in["k_cache"],
        "A_v_cache": _A_in["v_cache"],
        "A_wq": _A_in["wq"],
        "A_wo": _A_in["wo"],
        "B_x": _B_in["x"],
        "B_w_r": _B_in["w_r"],
        "B_w_gate": _B_in["w_gate"],
        "B_w_up": _B_in["w_up"],
        "B_w_down": _B_in["w_down"],
    }

def reference(A_x, A_k_cache, A_v_cache, A_wq, A_wo, B_x, B_w_r, B_w_gate, B_w_up, B_w_down):
    def _A_ref(x, k_cache, v_cache, wq, wo):
        B, Sq, D = x.shape
        Hq, Dh = 32, 128
        Hkv, Sk = k_cache.shape[1], k_cache.shape[2]
        W = min(4096, max(256, Sk // 4))
        rep = Hq // Hkv
        q = (lambda x, *d: x.transpose(*d))((x @ wq).reshape(B, Sq, Hq, Dh), 0, 2, 1, 3)
        k = jnp.repeat(k_cache[:, :, Sk - W:, :], rep, axis=1)
        v = jnp.repeat(v_cache[:, :, Sk - W:, :], rep, axis=1)
        scores = jnp.einsum("bhqd,bhkd->bhqk", q, k) * (Dh ** -0.5)
        p = _softmax(scores, axis=-1)
        o = jnp.einsum("bhqk,bhkd->bhqd", p, v)
        return (lambda x, *d: x.transpose(*d))(o, 0, 2, 1, 3).reshape(B, Sq, Hq * Dh) @ wo

    def _B_ref(x, w_r, w_gate, w_up, w_down):
        B, S, D = x.shape
        C = 1
        r = x @ w_r
        idx = jnp.argsort(-r, axis=-1)[:, :C]
        idx_e = jnp.repeat(idx.reshape(B, C, 1), D, axis=2)
        x_sel = jnp.take_along_axis(x, idx_e, axis=1)
        g = _silu(x_sel @ w_gate)
        u = x_sel @ w_up
        y = (g * u) @ w_down
        r_sel = _sigmoid(jnp.take_along_axis(r, idx, axis=1))
        y = y * r_sel.reshape(B, C, 1)
        b_off = (jnp.arange(B) * S).reshape(B, 1)
        flat_idx = (idx + b_off).reshape(B * C)
        zero = (x * 0.0).reshape(B * S, D)
        upd = _scatter_add(zero, flat_idx, y.reshape(B * C, D), axis=0)
        return x + upd.reshape(B, S, D)

    x = A_x
    xn = _layernorm(x, axis=-1)
    return x + _A_ref(xn, A_k_cache, A_v_cache, A_wq, A_wo) + _B_ref(xn, B_w_r, B_w_gate, B_w_up, B_w_down)
```

```python
import jax
import jax.numpy as jnp
from jax import lax
from jax.experimental import pallas as pl
from jax.experimental.pallas import tpu as pltpu

D = 512; HQ = 32; HKV = 8; DH = 128; F = 1792; REP = HQ // HKV

def build(cfg):
    window = cfg.get('window', 6)
    prio = cfg.get('prio', 1)
    kchunk = cfg.get('kchunk', 2048)
    wq_rows = cfg.get('wq_rows', 64)
    ffn_rows = cfg.get('ffn_rows', 128)
    wd_rows = cfg.get('wd_rows', 512)
    wo_rows = cfg.get('wo_rows', 512)
    M = cfg.get('M', 8)

    def kernel(x_hbm, k_hbm, v_hbm, wq_hbm, wo_hbm, wr_hbm, wg_hbm, wu_hbm, wd_hbm, out_ref,
               x_v, wr_v, wq_v, k_v, v_v, wo_v, wg_v, wu_v, wd_v, sems, sems_small):
        Sk = k_hbm.shape[2]
        W = min(4096, max(256, Sk // 4))
        W0 = Sk - W
        chunks = []
        marks = {}
        def add(tag, src, dst):
            chunks.append((src, dst))
        def mark(tag):
            marks[tag] = len(chunks)
        for r in range(0, D, wq_rows):
            add('wq', wq_hbm.at[pl.ds(r, wq_rows), :], wq_v.at[pl.ds(r, wq_rows), :])
            mark(('wq', r + wq_rows))
        for h in range(HKV):
            for r in range(0, W, kchunk):
                add('k', k_hbm.at[0, h, pl.ds(W0 + r, kchunk), :], k_v.at[h, pl.ds(r, kchunk), :])
            mark(('k', h))
        for h in range(HKV):
            for r in range(0, W, kchunk):
                add('v', v_hbm.at[0, h, pl.ds(W0 + r, kchunk), :], v_v.at[h, pl.ds(r, kchunk), :])
            mark(('v', h))
        for r in range(0, D, ffn_rows):
            add('wg', wg_hbm.at[pl.ds(r, ffn_rows), :], wg_v.at[pl.ds(r, ffn_rows), :])
            add('wu', wu_hbm.at[pl.ds(r, ffn_rows), :], wu_v.at[pl.ds(r, ffn_rows), :])
            mark(('ffn', r + ffn_rows))
        for r in range(0, F, wd_rows):
            n = min(wd_rows, F - r)
            add('wd', wd_hbm.at[pl.ds(r, n), :], wd_v.at[pl.ds(r, n), :])
            mark(('wd', r + n))
        for r in range(0, HQ * DH, wo_rows):
            add('wo', wo_hbm.at[pl.ds(r, wo_rows), :], wo_v.at[pl.ds(r, wo_rows), :])
            mark(('wo', r + wo_rows))
        n = len(chunks)
        state = dict(started=0, waited=0)
        def cp(i):
            return pltpu.make_async_copy(chunks[i][0], chunks[i][1], sems.at[i % window])
        def start_upto(m):
            while state['started'] < min(m, n):
                i = state['started']
                cp(i).start(priority=(i % 2) if prio else 0)
                state['started'] += 1
        def wait_upto(m):
            while state['waited'] < m:
                cp(state['waited']).wait()
                state['waited'] += 1
                start_upto(state['waited'] + window)
        def need(tag):
            wait_upto(marks[tag])

        cx = pltpu.make_async_copy(x_hbm, x_v, sems_small.at[0])
        cr = pltpu.make_async_copy(wr_hbm, wr_v, sems_small.at[1])
        cx.start(); cr.start()
        start_upto(window)
        cx.wait(); cr.wait()

        x = x_v[0].astype(jnp.float32)
        m = jnp.mean(x, axis=-1, keepdims=True)
        xc = x - m
        var = jnp.mean(xc * xc, axis=-1, keepdims=True)
        xn = xc / jnp.sqrt(var + 1e-5)
        xn_b = jnp.broadcast_to(xn, (M, D)).astype(jnp.bfloat16)
        wr = wr_v[...].astype(jnp.float32).reshape(1, D)
        r = jnp.sum(xn.astype(jnp.bfloat16).astype(jnp.float32) * wr, axis=-1, keepdims=True)
        r_sel = jax.nn.sigmoid(r)

        q = None
        for r0 in range(0, D, 128):
            need(('wq', r0 + 128))
            t = jnp.dot(xn_b[:, r0:r0 + 128], wq_v[pl.ds(r0, 128), :], preferred_element_type=jnp.float32)
            q = t if q is None else q + t
        q = q * (DH ** -0.5)
        row = lax.broadcasted_iota(jnp.int32, (M, DH), 0)
        rr = row % REP
        es = []; ls = []
        for h in range(HKV):
            t = [q[:, (REP * h + j) * DH:(REP * h + j + 1) * DH] for j in range(REP)]
            Qh = jnp.where(rr == 0, t[0], jnp.where(rr == 1, t[1], jnp.where(rr == 2, t[2], t[3]))).astype(jnp.bfloat16)
            need(('k', h))
            s = lax.dot_general(Qh, k_v[h], (((1,), (1,)), ((), ())), preferred_element_type=jnp.float32)
            mx = jnp.max(s, axis=-1, keepdims=True)
            e = jnp.exp(s - mx)
            ls.append(jnp.sum(e, axis=-1, keepdims=True))
            es.append(e.astype(jnp.bfloat16))
        os_ = []
        for h in range(HKV):
            need(('v', h))
            o = jnp.dot(es[h], v_v[h], preferred_element_type=jnp.float32)
            os_.append(o / ls[h])
        g = None; u = None
        for r0 in range(0, D, 128):
            need(('ffn', r0 + 128))
            tg = jnp.dot(xn_b[:, r0:r0 + 128], wg_v[pl.ds(r0, 128), :], preferred_element_type=jnp.float32)
            tu = jnp.dot(xn_b[:, r0:r0 + 128], wu_v[pl.ds(r0, 128), :], preferred_element_type=jnp.float32)
            g = tg if g is None else g + tg
            u = tu if u is None else u + tu
        hm = (g * jax.nn.sigmoid(g) * u).astype(jnp.bfloat16)
        y = None
        for r0 in range(0, F, wd_rows):
            nn = min(wd_rows, F - r0)
            need(('wd', r0 + nn))
            t = jnp.dot(hm[:, r0:r0 + nn], wd_v[pl.ds(r0, nn), :], preferred_element_type=jnp.float32)
            y = t if y is None else y + t
        base = x + xn + (xn * 0.0 + y[0:1] * r_sel)
        acc = None
        heads_per = wo_rows // DH
        for r0 in range(0, HQ * DH, wo_rows):
            hq0 = r0 // DH
            lhs = []
            for j in range(heads_per):
                hq = hq0 + j
                o = os_[hq // REP]
                lhs.append(jnp.broadcast_to(o[hq % REP:hq % REP + 1, :], (M, DH)))
            lhs = jnp.concatenate(lhs, axis=1).astype(jnp.bfloat16) if len(lhs) > 1 else lhs[0].astype(jnp.bfloat16)
            need(('wo', r0 + wo_rows))
            t = jnp.dot(lhs, wo_v[pl.ds(r0, wo_rows), :], preferred_element_type=jnp.float32)
            acc = t if acc is None else acc + t
        wait_upto(n)
        out = base + acc[0:1]
        out_ref[...] = out.astype(jnp.bfloat16).reshape(1, 1, D)

    @jax.jit
    def fn(A_x, A_k_cache, A_v_cache, A_wq, A_wo, B_x, B_w_r, B_w_gate, B_w_up, B_w_down):
        Sk = A_k_cache.shape[2]
        W = min(4096, max(256, Sk // 4))
        return pl.pallas_call(
            kernel,
            in_specs=[pl.BlockSpec(memory_space=pl.ANY)] * 9,
            out_specs=pl.BlockSpec(memory_space=pltpu.VMEM),
            out_shape=jax.ShapeDtypeStruct((1, 1, D), jnp.bfloat16),
            scratch_shapes=[
                pltpu.VMEM((1, 1, D), jnp.bfloat16), pltpu.VMEM((D,), jnp.bfloat16),
                pltpu.VMEM((D, HQ * DH), jnp.bfloat16),
                pltpu.VMEM((HKV, W, DH), jnp.bfloat16), pltpu.VMEM((HKV, W, DH), jnp.bfloat16),
                pltpu.VMEM((HQ * DH, D), jnp.bfloat16),
                pltpu.VMEM((D, F), jnp.bfloat16), pltpu.VMEM((D, F), jnp.bfloat16), pltpu.VMEM((F, D), jnp.bfloat16),
                pltpu.SemaphoreType.DMA((window,)), pltpu.SemaphoreType.DMA((2,)),
            ],
            compiler_params=pltpu.CompilerParams(vmem_limit_bytes=100 * 1024 * 1024, disable_bounds_checks=True),
            name=cfg.get('name', 'fused'),
        )(A_x, A_k_cache, A_v_cache, A_wq, A_wo, B_w_r, B_w_gate, B_w_up, B_w_down)
    return fn


_kernel_fn = build({'name': 'fused_decode'})


@jax.jit
def pallas_parallel_sum__sliding_block_cached__moe_arch_mod__decode_kernel(
    A_x, A_k_cache, A_v_cache, A_wq, A_wo, B_x, B_w_r, B_w_gate, B_w_up, B_w_down,
):
    return _kernel_fn(A_x, A_k_cache, A_v_cache, A_wq, A_wo, B_x, B_w_r, B_w_gate, B_w_up, B_w_down)
```

```python
import jax
import jax.numpy as jnp
from jax import lax
from jax.experimental import pallas as pl
from jax.experimental.pallas import tpu as pltpu
import contextlib

D = 512; HQ = 32; HKV = 8; DH = 128; F = 1792; REP = HQ // HKV
f32 = jnp.float32; bf16 = jnp.bfloat16

def build(cfg):
    w0 = cfg.get('w0', 8); w1 = cfg.get('w1', 8)
    kv_rows = cfg.get('kv_rows', 512); kv_p0 = cfg.get('kv_p0', 128)
    wq_mode = cfg.get('wq_mode', 'col')
    ff_rows = cfg.get('ff_rows', 32); ff_p0 = cfg.get('ff_p0', 8)
    dn_rows = 128; dn_p0 = cfg.get('dn_p0', 32)
    budget = cfg.get('budget', 100)
    order = cfg.get('order', 'qKVfo')
    M = 8
    scopes = cfg.get('scopes', False)
    ns = (lambda s: jax.named_scope(s)) if scopes else (lambda s: contextlib.nullcontext())
    nocompute = cfg.get('nocompute', False)

    def kernel(x_hbm, k_hbm, v_hbm, wq_hbm, wo_hbm, wr_hbm, wg_hbm, wu_hbm, wd_hbm, out_ref,
               x_v, wr_v, wq_v, k_v, v_v, wo_v, wg_v, wu_v, wd_v, sem0, sem1, sems_small):
        Sk = k_hbm.shape[2]
        W = min(4096, max(256, Sk // 4))
        W0 = Sk - W
        periods = []
        tasks = []
        st = {}
        def add_period(a, b):
            periods.append((a, b))
        def rows2(hbm, vm, r, n0, n):
            add_period((hbm.at[pl.ds(r, n0), :], vm.at[pl.ds(r, n0), :]),
                       (hbm.at[pl.ds(r + n0, n - n0), :], vm.at[pl.ds(r + n0, n - n0), :]))
        def task(cost, fn, name=''):
            tasks.append((len(periods) - 1, cost, fn, name))

        def wq_phase():
            for r0 in range(0, D, 128):
                if wq_mode == 'col':
                    for r in range(r0, r0 + 128, 16):
                        add_period((wq_hbm.at[pl.ds(r, 16), pl.ds(0, 1024)], wq_v.at[pl.ds(r, 16), pl.ds(0, 1024)]),
                                   (wq_hbm.at[pl.ds(r, 16), pl.ds(1024, 3072)], wq_v.at[pl.ds(r, 16), pl.ds(1024, 3072)]))
                elif wq_mode == 'row':
                    for r in range(r0, r0 + 128, 32):
                        rows2(wq_hbm, wq_v, r, 8, 32)
                elif wq_mode == 'row2':
                    for r in range(r0, r0 + 128, 16):
                        rows2(wq_hbm, wq_v, r, 8, 16)
                for j in range(8):
                    def fn(r0=r0, j=j):
                        t = jnp.dot(st['xn_b'][:, r0:r0 + 128], wq_v[pl.ds(r0, 128), pl.ds(512 * j, 512)], preferred_element_type=f32)
                        st['q', j] = t if r0 == 0 else st['q', j] + t
                    task(32, fn, f'q{r0}_{j}')
        nb = W // kv_rows
        def k_head(h):
            for b in range(nb):
                rows2(k_hbm.at[0, h], k_v.at[h], W0 + b * kv_rows, kv_p0, kv_rows) if False else None
                r = b * kv_rows
                add_period((k_hbm.at[0, h, pl.ds(W0 + r, kv_p0), :], k_v.at[h, pl.ds(r, kv_p0), :]),
                           (k_hbm.at[0, h, pl.ds(W0 + r + kv_p0, kv_rows - kv_p0), :], k_v.at[h, pl.ds(r + kv_p0, kv_rows - kv_p0), :]))
                def fn(h=h, b=b, r=r):
                    if b == 0:
                        q = st['q', h] * (DH ** -0.5)
                        row = lax.broadcasted_iota(jnp.int32, (M, DH), 0) % REP
                        t = [q[:, j * DH:(j + 1) * DH] for j in range(REP)]
                        st['Q', h] = jnp.where(row == 0, t[0], jnp.where(row == 1, t[1], jnp.where(row == 2, t[2], t[3]))).astype(bf16)
                    s = lax.dot_general(st['Q', h], k_v[h, pl.ds(r, kv_rows), :], (((1,), (1,)), ((), ())), preferred_element_type=f32)
                    st['s', h, b] = s
                    mx = s if b == 0 else jnp.maximum(st['mx', h], s)
                    st['mx', h] = mx
                task(32 * kv_rows // 512 + 8, fn, f's{h}_{b}')
        def v_head(h):
            for b in range(nb):
                r = b * kv_rows
                add_period((v_hbm.at[0, h, pl.ds(W0 + r, kv_p0), :], v_v.at[h, pl.ds(r, kv_p0), :]),
                           (v_hbm.at[0, h, pl.ds(W0 + r + kv_p0, kv_rows - kv_p0), :], v_v.at[h, pl.ds(r + kv_p0, kv_rows - kv_p0), :]))
                def fn(h=h, b=b, r=r):
                    if b == 0:
                        st['m', h] = jnp.max(st['mx', h], axis=-1, keepdims=True)
                    e = jnp.exp(st['s', h, b] - st['m', h])
                    st['ls', h] = e if b == 0 else st['ls', h] + e
                    t = jnp.dot(e.astype(bf16), v_v[h, pl.ds(r, kv_rows), :], preferred_element_type=f32)
                    st['o', h] = t if b == 0 else st['o', h] + t
                    if b == nb - 1:
                        l = jnp.sum(st['ls', h], axis=-1, keepdims=True)
                        st['o', h] = st['o', h] / l
                task(32 * kv_rows // 512 + 24, fn, f'pv{h}_{b}')
        def ffn_up():
            for r0 in range(0, D, 128):
                for nm, hbm, vm in (('g', wg_hbm, wg_v), ('u', wu_hbm, wu_v)):
                    for r in range(r0, r0 + 128, ff_rows):
                        rows2(hbm, vm, r, ff_p0, ff_rows)
                    for c0 in range(0, F, 512):
                        cn = min(512, F - c0)
                        def fn(nm=nm, vm=vm, r0=r0, c0=c0, cn=cn):
                            t = jnp.dot(st['xn_b'][:, r0:r0 + 128], vm[pl.ds(r0, 128), pl.ds(c0, cn)], preferred_element_type=f32)
                            st[nm, c0] = t if r0 == 0 else st[nm, c0] + t
                        task(32, fn, f'{nm}{r0}_{c0}')
        def ffn_down():
            for r in range(0, F, dn_rows):
                rows2(wd_hbm, wd_v, r, dn_p0, dn_rows)
                def fn(r=r):
                    c0 = (r // 512) * 512
                    if ('hm', c0) not in st:
                        g = st['g', c0]; u = st['u', c0]
                        st['hm', c0] = (g * jax.nn.sigmoid(g) * u).astype(bf16)
                    t = jnp.dot(st['hm', c0][:, r - c0:r - c0 + dn_rows], wd_v[pl.ds(r, dn_rows), :], preferred_element_type=f32)
                    st['y'] = t if r == 0 else st['y'] + t
                task(40, fn, f'd{r}')
        def wo_phase():
            for r in range(0, HQ * DH, dn_rows):
                rows2(wo_hbm, wo_v, r, dn_p0, dn_rows)
                def fn(r=r):
                    hq = r // DH
                    o = st['o', hq // REP]
                    lhs = jnp.broadcast_to(o[hq % REP:hq % REP + 1, :], (M, DH)).astype(bf16)
                    t = jnp.dot(lhs, wo_v[pl.ds(r, dn_rows), :], preferred_element_type=f32)
                    st['acc'] = t if r == 0 else st['acc'] + t
                task(40, fn, f'o{r}')
        for ch in order:
            if ch == 'q': wq_phase()
            elif ch == 'K':
                for h in range(HKV): k_head(h)
            elif ch == 'V':
                for h in range(HKV): v_head(h)
            elif ch == 'A':
                for h in range(HKV):
                    k_head(h); v_head(h)
            elif ch == 'f': ffn_up(); ffn_down()
            elif ch == 'o': wo_phase()
        n = len(periods)
        def cp(s, i):
            ring, w = (sem0, w0) if s == 0 else (sem1, w1)
            return pltpu.make_async_copy(periods[i][s][0], periods[i][s][1], ring.at[i % w])

        cx = pltpu.make_async_copy(x_hbm, x_v, sems_small.at[0])
        cr = pltpu.make_async_copy(wr_hbm, wr_v, sems_small.at[1])
        with ns('issue'):
            cp(1, 0).start(priority=1)
            cx.start(); cr.start()
            cp(0, 0).start(priority=0)
            for i in range(1, max(w0, w1)):
                if i < w1: cp(1, i).start(priority=1)
                if i < w0: cp(0, i).start(priority=0)
        with ns('wait_x'):
            cx.wait(); cr.wait()
        with ns('ln'):
            x = x_v[0].astype(f32)
            m = jnp.mean(x, axis=-1, keepdims=True)
            xc = x - m
            var = jnp.mean(xc * xc, axis=-1, keepdims=True)
            xn = xc / jnp.sqrt(var + 1e-5)
            st['xn_b'] = jnp.broadcast_to(xn, (M, D)).astype(bf16)
            wr = wr_v[...].astype(f32).reshape(1, D)
            r = jnp.sum(xn.astype(bf16).astype(f32) * wr, axis=-1, keepdims=True)
            r_sel = jax.nn.sigmoid(r)
        ti = 0
        for i in range(n):
            with ns(f'w{i}'):
                cp(0, i).wait()
                if i + w0 < n: cp(0, i + w0).start(priority=0)
                cp(1, i).wait()
                if i + w1 < n: cp(1, i + w1).start(priority=1)
            b = budget
            while not nocompute and ti < len(tasks) and tasks[ti][0] <= i and (b >= tasks[ti][1] or b == budget or i == n - 1):
                with ns(tasks[ti][3]):
                    tasks[ti][2]()
                b -= tasks[ti][1]; ti += 1
        with ns('final'):
            if nocompute:
                out = x + xn + wo_v[0:1, :].astype(f32) + r_sel
            else:
                assert ti == len(tasks)
                base = x + xn + (xn * 0.0 + st['y'][0:1] * r_sel)
                out = base + st['acc'][0:1]
            out_ref[...] = out.astype(bf16).reshape(1, 1, D)

    @jax.jit
    def fn(A_x, A_k_cache, A_v_cache, A_wq, A_wo, B_x, B_w_r, B_w_gate, B_w_up, B_w_down):
        Sk = A_k_cache.shape[2]
        W = min(4096, max(256, Sk // 4))
        return pl.pallas_call(
            kernel,
            in_specs=[pl.BlockSpec(memory_space=pl.ANY)] * 9,
            out_specs=pl.BlockSpec(memory_space=pltpu.VMEM),
            out_shape=jax.ShapeDtypeStruct((1, 1, D), bf16),
            scratch_shapes=[
                pltpu.VMEM((1, 1, D), bf16), pltpu.VMEM((D,), bf16),
                pltpu.VMEM((D, HQ * DH), bf16),
                pltpu.VMEM((HKV, W, DH), bf16), pltpu.VMEM((HKV, W, DH), bf16),
                pltpu.VMEM((HQ * DH, D), bf16),
                pltpu.VMEM((D, F), bf16), pltpu.VMEM((D, F), bf16), pltpu.VMEM((F, D), bf16),
                pltpu.SemaphoreType.DMA((w0,)), pltpu.SemaphoreType.DMA((w1,)), pltpu.SemaphoreType.DMA((2,)),
            ],
            compiler_params=pltpu.CompilerParams(vmem_limit_bytes=100 * 1024 * 1024, disable_bounds_checks=True,
                                                 disable_semaphore_checks=cfg.get('nosemchk', True)),
            name=cfg.get('name', 'fused'),
        )(A_x, A_k_cache, A_v_cache, A_wq, A_wo, B_w_r, B_w_gate, B_w_up, B_w_down)
    return fn


_CFG = {'w0': 10, 'w1': 12}
_CFG['name'] = 'fused_decode'
_kernel_fn = build(_CFG)


@jax.jit
def pallas_parallel_sum__sliding_block_cached__moe_arch_mod__decode_kernel(
    A_x, A_k_cache, A_v_cache, A_wq, A_wo, B_x, B_w_r, B_w_gate, B_w_up, B_w_down,
):
    return _kernel_fn(A_x, A_k_cache, A_v_cache, A_wq, A_wo, B_x, B_w_r, B_w_gate, B_w_up, B_w_down)
```

```python
import jax
import jax.numpy as jnp
from jax import lax
from jax.experimental import pallas as pl
from jax.experimental.pallas import tpu as pltpu
import contextlib
import bisect

D = 512; HQ = 32; HKV = 8; DH = 128; F = 1792; REP = HQ // HKV
f32 = jnp.float32; bf16 = jnp.bfloat16

PLANS = {
    'P4': ([('wg', None, 0, 512), ('wu', None, 0, 512), ('wd', None, 0, 1792), ('wo', None, 0, 3072)],
           [('wq', None, 0, 512)] + [('k', h, 0, 4096) for h in range(8)] + [('v', h, 0, 4096) for h in range(8)] + [('wo', None, 3072, 4096)]),
    'P5': ([('v', h, 0, 4096) for h in range(8)],
           [('wq', None, 0, 512)] + [('k', h, 0, 4096) for h in range(8)] + [('wg', None, 0, 512), ('wu', None, 0, 512), ('wd', None, 0, 1792), ('wo', None, 0, 4096)]),
    'P2': ([('wg', None, 0, 512), ('wu', None, 0, 512), ('wd', None, 0, 1792)] + [('v', h, 0, 4096) for h in range(3)],
           [('wq', None, 0, 512)] + [('k', h, 0, 4096) for h in range(8)] + [('v', h, 0, 4096) for h in range(3, 8)] + [('wo', None, 0, 4096)]),
    'P1': ([('v', h, 0, 4096) for h in range(3)] + [('wg', None, 0, 512), ('wu', None, 0, 512), ('wd', None, 0, 1792)],
           [('wq', None, 0, 512)] + [('k', h, 0, 4096) for h in range(8)] + [('v', h, 0, 4096) for h in range(3, 8)] + [('wo', None, 0, 4096)]),
}
ROWB = {'wq': 8192, 'wo': 1024, 'wd': 1024, 'wg': 3584, 'wu': 3584, 'k': 256, 'v': 256}

def build(cfg):
    w0 = cfg.get('w0', 8); w1 = cfg.get('w1', 8)
    c0 = cfg.get('c0', 32) * 1024; c1 = cfg.get('c1', 96) * 1024
    plan = PLANS[cfg.get('plan', 'P4')]
    budget = cfg.get('budget', 40)
    M = 8
    scopes = cfg.get('scopes', False)
    ns = (lambda s: jax.named_scope(s)) if scopes else (lambda s: contextlib.nullcontext())
    tail_scopes = cfg.get('tail_scopes', 0)
    nst = lambda s, on: jax.named_scope(s) if on else contextlib.nullcontext()
    nocompute = cfg.get('nocompute', False)
    lead0 = cfg.get('lead0', 0.0)

    def kernel(x_hbm, k_hbm, v_hbm, wq_hbm, wo_hbm, wr_hbm, wg_hbm, wu_hbm, wd_hbm, out_ref,
               x_v, wr_v, wq_v, k_v, v_v, wo_v, wg_v, wu_v, wd_v, sem0, sem1, sems_small, semt):
        Sk = k_hbm.shape[2]
        W = min(4096, max(256, Sk // 4))
        W0 = Sk - W
        assert W == 4096
        hbm = dict(wq=wq_hbm, wo=wo_hbm, wg=wg_hbm, wu=wu_hbm, wd=wd_hbm, k=k_hbm, v=v_hbm)
        vm = dict(wq=wq_v, wo=wo_v, wg=wg_v, wu=wu_v, wd=wd_v, k=k_v, v=v_v)
        S = [[], []]
        tp = cfg.get('tp', 0)
        TR = cfg.get('trows', 128)
        R0 = HQ * DH - (TR if tp else 0)
        where = {}
        for s in (0, 1):
            cb = (c0, c1)[s]
            for (nm, h, a, b) in plan[s]:
                if nm == 'wo' and s == 1: b = min(b, R0)
                rows = max(8, (cb // ROWB[nm]) // 8 * 8)
                if s == 1 and nm == 'wo' and cfg.get('wo_rows1'): rows = cfg['wo_rows1']
                if s == 1 and nm == 'wq' and cfg.get('wq_rows1'): rows = cfg['wq_rows1']
                for r in range(a, b, rows):
                    n = min(rows, b - r)
                    S[s].append((nm, h, r, n))
                    where.setdefault((nm, h), []).append((r, r + n, s, len(S[s])))
        def dep(nm, h, r0, r1):
            need = [0, 0]
            for (a, b, s, cnt) in where[(nm, h)]:
                if a < r1 and b > r0:
                    need[s] = max(need[s], cnt)
            return tuple(need)
        n0, n1 = len(S[0]), len(S[1])
        Wn = (min(w0, n0), min(w1, n1))
        def cp(s, i):
            nm, h, r, n = S[s][i]
            ring = (sem0, sem1)[s]
            if h is not None:
                return pltpu.make_async_copy(hbm[nm].at[0, h, pl.ds(W0 + r, n), :], vm[nm].at[h, pl.ds(r, n), :], ring.at[i % Wn[s]])
            return pltpu.make_async_copy(hbm[nm].at[pl.ds(r, n), :], vm[nm].at[pl.ds(r, n), :], ring.at[i % Wn[s]])
        def cum(L):
            t = 0; out = []
            for (nm, h, r, n) in L:
                t += n * ROWB[nm]; out.append(t)
            return [x / t for x in out]
        b0, b1 = cum(S[0]), cum(S[1])
        order = []; i0 = i1 = 0
        while i0 < n0 or i1 < n1:
            f0 = b0[i0] - lead0 if i0 < n0 else 9; f1 = b1[i1] if i1 < n1 else 9
            if f0 <= f1: order.append((0, i0)); i0 += 1
            else: order.append((1, i1)); i1 += 1
        st = {}
        tasks = []
        def task(name, deps, after, cost, fn):
            tasks.append((name, deps, after, cost, fn))
        for r0 in range(0, D, 128):
            for j in range(8):
                def fn(r0=r0, j=j):
                    t = jnp.dot(st['xn_b'][:, r0:r0 + 128], wq_v[pl.ds(r0, 128), pl.ds(512 * j, 512)], preferred_element_type=f32)
                    st['q', j] = t if r0 == 0 else st['q', j] + t
                task(f'q{r0}_{j}', dep('wq', None, r0, r0 + 128), [f'q{r0-128}_{j}'] if r0 else [], 32, fn)
        KB = cfg.get('kb', 512)
        nb = W // KB
        for h in range(HKV):
            for b in range(nb):
                r = b * KB
                def fn(h=h, b=b, r=r):
                    if b == 0:
                        q = st['q', h] * (DH ** -0.5)
                        row = lax.broadcasted_iota(jnp.int32, (M, DH), 0) % REP
                        t = [q[:, j * DH:(j + 1) * DH] for j in range(REP)]
                        st['Q', h] = jnp.where(row == 0, t[0], jnp.where(row == 1, t[1], jnp.where(row == 2, t[2], t[3]))).astype(bf16)
                    s = lax.dot_general(st['Q', h], k_v[h, pl.ds(r, KB), :], (((1,), (1,)), ((), ())), preferred_element_type=f32)
                    st['s', h, b] = s
                    st['mx', h] = s if b == 0 else jnp.maximum(st['mx', h], s)
                task(f's{h}_{b}', dep('k', h, r, r + KB), [f'q384_{h}'] if b == 0 else [f's{h}_{b-1}'], 32 * KB // 512, fn)
        for h in range(HKV):
            for b in range(nb):
                r = b * KB
                def fn(h=h, b=b, r=r):
                    if b == 0:
                        st['m', h] = jnp.max(st['mx', h], axis=-1, keepdims=True)
                    e = jnp.exp(st['s', h, b] - st['m', h])
                    st['ls', h] = e if b == 0 else st['ls', h] + e
                    t = jnp.dot(e.astype(bf16), v_v[h, pl.ds(r, KB), :], preferred_element_type=f32)
                    st['o', h] = t if b == 0 else st['o', h] + t
                    if b == nb - 1:
                        l = jnp.sum(st['ls', h], axis=-1, keepdims=True)
                        st['o', h] = st['o', h] / l
                task(f'pv{h}_{b}', dep('v', h, r, r + KB), [f's{h}_{nb-1}'] if b == 0 else [f'pv{h}_{b-1}'], 32 * KB // 512, fn)
        for r0 in range(0, D, 128):
            for nm, key in (('wg', 'g'), ('wu', 'u')):
                for c in range(0, F, 512):
                    cn = min(512, F - c)
                    def fn(nm=nm, key=key, r0=r0, c=c, cn=cn):
                        t = jnp.dot(st['xn_b'][:, r0:r0 + 128], vm[nm][pl.ds(r0, 128), pl.ds(c, cn)], preferred_element_type=f32)
                        st[key, c] = t if r0 == 0 else st[key, c] + t
                    task(f'{key}{r0}_{c}', dep(nm, None, r0, r0 + 128), [f'{key}{r0-128}_{c}'] if r0 else [], 32, fn)
        for r in range(0, F, 128):
            c = (r // 512) * 512
            def fn(r=r, c=c):
                if ('hm', c) not in st:
                    g = st['g', c]; u = st['u', c]
                    st['hm', c] = (g * jax.nn.sigmoid(g) * u).astype(bf16)
                t = jnp.dot(st['hm', c][:, r - c:r - c + 128], wd_v[pl.ds(r, 128), :], preferred_element_type=f32)
                st['y'] = t if r == 0 else st['y'] + t
            task(f'd{r}', dep('wd', None, r, r + 128), [f'g384_{c}', f'u384_{c}'] + ([f'd{r-128}'] if r else []), 32, fn)
        for r in range(0, R0, 128):
            hq = r // DH
            kk = min(128, R0 - r)
            def fn(r=r, hq=hq, kk=kk):
                o = st['o', hq // REP]
                lhs = jnp.broadcast_to(o[hq % REP:hq % REP + 1, 0:kk], (M, kk)).astype(bf16)
                t = jnp.dot(lhs, wo_v[pl.ds(r, kk), :], preferred_element_type=f32)
                st['acc'] = t if 'acc' not in st else st['acc'] + t
            task(f'o{r}', dep('wo', None, r, r + kk), [f'pv{hq // REP}_{nb-1}'], 32, fn)
        if tp:
            def fn():
                o = st['o', HKV - 1]
                a = o[REP - 1:REP, :].astype(bf16).astype(f32)
                st['AT'] = jnp.transpose(jnp.broadcast_to(a, (DH, DH)))
            task('AT', (0, 0), [f'pv{HKV-1}_{nb-1}'], 16, fn)

        cx = pltpu.make_async_copy(x_hbm, x_v, sems_small.at[0])
        cr = pltpu.make_async_copy(wr_hbm, wr_v, sems_small.at[1])
        started = [0, 0]
        with ns('issue'):
            first = True
            for s, i in order:
                if started[s] < Wn[s]:
                    cp(s, started[s]).start(priority=s); started[s] += 1
                if first:
                    cx.start(); cr.start(); first = False
                if started[0] >= Wn[0] and started[1] >= Wn[1]: break
        with ns('wait_x'):
            cx.wait(); cr.wait()
        with ns('ln'):
            x = x_v[0].astype(f32)
            m = jnp.mean(x, axis=-1, keepdims=True)
            xc = x - m
            var = jnp.mean(xc * xc, axis=-1, keepdims=True)
            xn = xc / jnp.sqrt(var + 1e-5)
            st['xn_b'] = jnp.broadcast_to(xn, (M, D)).astype(bf16)
            wr = wr_v[...].astype(f32).reshape(1, D)
            r = jnp.sum(xn.astype(bf16).astype(f32) * wr, axis=-1, keepdims=True)
            r_sel = jax.nn.sigmoid(r)
        done = set(); pending = list(tasks); waited = [0, 0]
        fk = []
        def run_ready(b, flush=False):
            run_ready_(b, flush)
            if fk:
                pl.delay(cfg['fake'] + sum(fk)); fk.clear()
        def run_ready_(b, flush=False):
            progress = True
            while progress and not nocompute:
                progress = False
                for t in pending:
                    name, deps, after, cost, fn = t
                    if deps[0] <= waited[0] and deps[1] <= waited[1] and all(a in done for a in after):
                        if not flush and b < cost and b != budget: return
                        with ns(name):
                            if cfg.get('fake'):
                                fk.append(cost)
                            else:
                                fn()
                        b -= cost; done.add(name); pending.remove(t); progress = True
                        break
        periods = []
        i0 = 0
        for i1 in range(n1):
            ev = [(1, i1)]
            while i0 < n0 and (b0[i0] - lead0 <= b1[i1] or i1 == n1 - 1):
                ev.append((0, i0)); i0 += 1
            if cfg.get('p0first', False): ev = ev[1:] + ev[:1]
            periods.append(ev)
        pair = cfg.get('pair', 2)
        asap_tail = cfg.get('asap_tail', 4)
        def n_ready():
            c = 0; d = set(done)
            for t in pending:
                name, deps, after, cost, fn = t
                if deps[0] <= waited[0] and deps[1] <= waited[1] and all(a in d for a in after):
                    c += 1; d.add(name)
            return c
        def cpt(j):
            r = R0 + j * tp
            return pltpu.make_async_copy(wo_hbm.at[pl.ds(r, tp), :], wo_v.at[pl.ds(r, tp), :], semt.at[j])
        ntp = TR // tp if tp else 0
        tail_started = [False]
        for pi, ev in enumerate(periods):
            for (s, i) in ev:
                with ns(f'w{s}_{i}'):
                    with nst(f'T{s}_{i}', pi >= len(periods) - tail_scopes):
                        cp(s, i).wait(); waited[s] += 1
                    if started[s] < len(S[s]):
                        cp(s, started[s]).start(priority=s); started[s] += 1
                    elif s == 1 and tp and not tail_started[0]:
                        tail_started[0] = True
                        for j in range(ntp): cpt(j).start(priority=1)
            if pi == len(periods) - 1:
                run_ready(budget, flush=True)
            elif pi >= len(periods) - asap_tail or n_ready() >= pair:
                run_ready(budget)
        with ns('final'):
            if nocompute or cfg.get('fake'):
                for j in range(ntp): cpt(j).wait()
                out = x + xn + wo_v[0:1, :].astype(f32) + r_sel
            else:
                assert not pending, [p[0] for p in pending]
                base = x + xn + (xn * 0.0 + st['y'][0:1] * r_sel)
                out = base + st['acc'][0:1]
                if tp:
                    assert tail_started[0]
                    AT = st['AT']
                    av = None
                    k0 = R0 - (HQ - 1) * DH
                    for j in range(ntp):
                        with nst(f'TT{j}', tail_scopes > 0):
                            cpt(j).wait()
                        w = wo_v[pl.ds(R0 + j * tp, tp), :].astype(f32)
                        a = AT[k0 + j * tp:k0 + (j + 1) * tp, :]
                        p = [w[:, c * DH:(c + 1) * DH] * a for c in range(D // DH)]
                        p = jnp.concatenate(p, axis=1)
                        for q in range(0, tp, 8):
                            av = p[q:q + 8] if av is None else av + p[q:q + 8]
                    out = out + jnp.sum(av, axis=0, keepdims=True)
            out_ref[...] = out.astype(bf16).reshape(1, 1, D)

    @jax.jit
    def fn(A_x, A_k_cache, A_v_cache, A_wq, A_wo, B_x, B_w_r, B_w_gate, B_w_up, B_w_down):
        Sk = A_k_cache.shape[2]
        W = min(4096, max(256, Sk // 4))
        return pl.pallas_call(
            kernel,
            in_specs=[pl.BlockSpec(memory_space=pl.ANY)] * 9,
            out_specs=pl.BlockSpec(memory_space=pltpu.VMEM),
            out_shape=jax.ShapeDtypeStruct((1, 1, D), bf16),
            scratch_shapes=[
                pltpu.VMEM((1, 1, D), bf16), pltpu.VMEM((D,), bf16),
                pltpu.VMEM((D, HQ * DH), bf16),
                pltpu.VMEM((HKV, W, DH), bf16), pltpu.VMEM((HKV, W, DH), bf16),
                pltpu.VMEM((HQ * DH, D), bf16),
                pltpu.VMEM((D, F), bf16), pltpu.VMEM((D, F), bf16), pltpu.VMEM((F, D), bf16),
                pltpu.SemaphoreType.DMA((w0,)), pltpu.SemaphoreType.DMA((w1,)), pltpu.SemaphoreType.DMA((2,)), pltpu.SemaphoreType.DMA((max(1, cfg.get('trows', 128) // max(cfg.get('tp', 0), 1)),)),
            ],
            compiler_params=pltpu.CompilerParams(vmem_limit_bytes=100 * 1024 * 1024, disable_bounds_checks=True,
                                                 disable_semaphore_checks=cfg.get('nosemchk', True)),
            name=cfg.get('name', 'fused'),
        )(A_x, A_k_cache, A_v_cache, A_wq, A_wo, B_w_r, B_w_gate, B_w_up, B_w_down)
    return fn


_CFG = {'plan': 'P4', 'w0': 12, 'w1': 10, 'budget': 64, 'lead0': 0.02, 'pair': 2, 'wo_rows1': 128, 'tp': 16, 'trows': 128}
_CFG['name'] = 'fused_decode'
_kernel_fn = build(_CFG)


@jax.jit
def pallas_parallel_sum__sliding_block_cached__moe_arch_mod__decode_kernel(
    A_x, A_k_cache, A_v_cache, A_wq, A_wo, B_x, B_w_r, B_w_gate, B_w_up, B_w_down,
):
    return _kernel_fn(A_x, A_k_cache, A_v_cache, A_wq, A_wo, B_x, B_w_r, B_w_gate, B_w_up, B_w_down)
```

```python
import jax
import jax.numpy as jnp
from jax import lax
from jax.experimental import pallas as pl
from jax.experimental.pallas import tpu as pltpu

D = 512
HQ = 32
HKV = 8
DH = 128
F = 1792
REP = HQ // HKV
M = 8

ROW_BYTES = {"wq": 2 * HQ * DH, "wo": 2 * D, "wd": 2 * D, "wg": 2 * F, "wu": 2 * F, "k": 2 * DH, "v": 2 * DH}
CHUNK_BYTES = (32 * 1024, 96 * 1024)
IN_FLIGHT = (12, 12)
Q0_LEAD = 0.02
WO_Q1_ROWS = 128
TAIL_ROWS = 128
TAIL_PIECE = 16
KEY_BLOCK = 512
LN_PERIOD = 3
TASKS_PER_PERIOD = 2
EAGER_PERIODS = 4


def _streams(window):
  tail0 = HQ * DH - TAIL_ROWS
  wo_split = 3 * HQ * DH // 4
  heads = range(HKV)
  plan = (
      [("wg", None, 0, D), ("wu", None, 0, D), ("wd", None, 0, F), ("wo", None, 0, wo_split)],
      [("wq", None, 0, D)]
      + [("k", h, 0, window) for h in heads]
      + [("v", h, 0, window) for h in heads]
      + [("wo", None, wo_split, tail0)],
  )
  streams = ([], [])
  for q in (0, 1):
    for name, head, lo, hi in plan[q]:
      rows = max(8, CHUNK_BYTES[q] // ROW_BYTES[name] // 8 * 8)
      if q == 1 and name == "wo":
        rows = WO_Q1_ROWS
      for r in range(lo, hi, rows):
        streams[q].append((name, head, r, min(rows, hi - r)))
  return streams


def _periods(streams):
  frac = []
  for chunks in streams:
    acc, cum = 0, []
    for name, _, _, rows in chunks:
      acc += rows * ROW_BYTES[name]
      cum.append(acc)
    frac.append([c / acc for c in cum])
  n0, n1 = len(streams[0]), len(streams[1])
  periods, j = [], 0
  for i in range(n1):
    events = [(1, i)]
    while j < n0 and (frac[0][j] - Q0_LEAD <= frac[1][i] or i == n1 - 1):
      events.append((0, j))
      j += 1
    periods.append(events)
  return periods


def _kernel(x_hbm, k_hbm, v_hbm, wq_hbm, wo_hbm, wr_hbm, wg_hbm, wu_hbm, wd_hbm, out_ref,
            x_v, wr_v, wq_v, k_v, v_v, wo_v, wg_v, wu_v, wd_v, sem_q0, sem_q1, sem_small, sem_tail):
  f32, bf16 = jnp.float32, jnp.bfloat16
  seq = k_hbm.shape[2]
  window = min(4096, max(256, seq // 4))
  w0 = seq - window
  hbm = dict(wq=wq_hbm, wo=wo_hbm, wg=wg_hbm, wu=wu_hbm, wd=wd_hbm, k=k_hbm, v=v_hbm)
  vmem = dict(wq=wq_v, wo=wo_v, wg=wg_v, wu=wu_v, wd=wd_v, k=k_v, v=v_v)
  streams = _streams(window)
  periods = _periods(streams)
  tail0 = HQ * DH - TAIL_ROWS
  n_tail = TAIL_ROWS // TAIL_PIECE
  n_kb = window // KEY_BLOCK

  def copy(q, i):
    name, head, r, rows = streams[q][i]
    sem = (sem_q0, sem_q1)[q].at[i % IN_FLIGHT[q]]
    if head is None:
      return pltpu.make_async_copy(hbm[name].at[pl.ds(r, rows), :], vmem[name].at[pl.ds(r, rows), :], sem)
    return pltpu.make_async_copy(hbm[name].at[0, head, pl.ds(w0 + r, rows), :],
                                 vmem[name].at[head, pl.ds(r, rows), :], sem)

  def tail_copy(j):
    rows = pl.ds(tail0 + j * TAIL_PIECE, TAIL_PIECE)
    return pltpu.make_async_copy(wo_hbm.at[rows, :], wo_v.at[rows, :], sem_tail.at[j])

  def needs(name, head, lo, hi):
    need = [0, 0]
    for q in (0, 1):
      for i, (n, h, r, rows) in enumerate(streams[q]):
        if n == name and h == head and r < hi and r + rows > lo:
          need[q] = max(need[q], i + 1)
    return tuple(need)

  st = {}
  tasks = []

  def layernorm_mean():
    x_copy.wait()
    st["x"] = x_v[0].astype(f32)
    st["xc"] = st["x"] - jnp.mean(st["x"], axis=-1, keepdims=True)

  def layernorm_scale():
    var = jnp.mean(st["xc"] * st["xc"], axis=-1, keepdims=True)
    st["xn"] = st["xc"] / jnp.sqrt(var + 1e-5)
    st["xn_b"] = jnp.broadcast_to(st["xn"], (M, D)).astype(bf16)

  def router():
    wr_copy.wait()
    w_r = wr_v[...].astype(f32).reshape(1, D)
    r = jnp.sum(st["xn"].astype(bf16).astype(f32) * w_r, axis=-1, keepdims=True)
    st["r_sel"] = jax.nn.sigmoid(r)

  def accumulate(key, val):
    st[key] = val if key not in st else st[key] + val

  for r in range(0, D, 128):
    for h in range(HKV):
      def q_proj(r=r, h=h):
        accumulate(("q", h), jnp.dot(st["xn_b"][:, r:r + 128], wq_v[pl.ds(r, 128), pl.ds(REP * DH * h, REP * DH)],
                                     preferred_element_type=f32))
      tasks.append((f"q{r}_{h}", needs("wq", None, r, r + 128), [f"q{r - 128}_{h}"] if r else [], q_proj))

  for h in range(HKV):
    for b in range(n_kb):
      def scores(h=h, b=b):
        if b == 0:
          q = st["q", h] * (DH ** -0.5)
          row = lax.broadcasted_iota(jnp.int32, (M, DH), 0) % REP
          t = [q[:, j * DH:(j + 1) * DH] for j in range(REP)]
          st["qh", h] = jnp.where(row == 0, t[0], jnp.where(row == 1, t[1], jnp.where(row == 2, t[2], t[3]))).astype(bf16)
        s = lax.dot_general(st["qh", h], k_v[h, pl.ds(b * KEY_BLOCK, KEY_BLOCK), :], (((1,), (1,)), ((), ())),
                            preferred_element_type=f32)
        st["s", h, b] = s
        st["smax", h] = s if b == 0 else jnp.maximum(st["smax", h], s)
      tasks.append((f"s{h}_{b}", needs("k", h, b * KEY_BLOCK, (b + 1) * KEY_BLOCK),
                    [f"q{D - 128}_{h}"] if b == 0 else [f"s{h}_{b - 1}"], scores))

  for h in range(HKV):
    for b in range(n_kb):
      def attend(h=h, b=b):
        if b == 0:
          st["m", h] = jnp.max(st["smax", h], axis=-1, keepdims=True)
        e = jnp.exp(st["s", h, b] - st["m", h])
        accumulate(("esum", h), e)
        accumulate(("o", h), jnp.dot(e.astype(bf16), v_v[h, pl.ds(b * KEY_BLOCK, KEY_BLOCK), :],
                                     preferred_element_type=f32))
        if b == n_kb - 1:
          st["o", h] = st["o", h] / jnp.sum(st["esum", h], axis=-1, keepdims=True)
      tasks.append((f"pv{h}_{b}", needs("v", h, b * KEY_BLOCK, (b + 1) * KEY_BLOCK),
                    [f"s{h}_{n_kb - 1}"] if b == 0 else [f"pv{h}_{b - 1}"], attend))

  for r in range(0, D, 128):
    for name in ("wg", "wu"):
      for c in range(0, F, 512):
        def up_proj(name=name, r=r, c=c):
          accumulate((name, c), jnp.dot(st["xn_b"][:, r:r + 128], vmem[name][pl.ds(r, 128), pl.ds(c, min(512, F - c))],
                                        preferred_element_type=f32))
        tasks.append((f"{name}{r}_{c}", needs(name, None, r, r + 128), [f"{name}{r - 128}_{c}"] if r else [], up_proj))

  for r in range(0, F, 128):
    c = r // 512 * 512
    def down_proj(r=r, c=c):
      if ("h", c) not in st:
        g = st["wg", c]
        st["h", c] = (g * jax.nn.sigmoid(g) * st["wu", c]).astype(bf16)
      accumulate("y", jnp.dot(st["h", c][:, r - c:r - c + 128], wd_v[pl.ds(r, 128), :], preferred_element_type=f32))
    tasks.append((f"d{r}", needs("wd", None, r, r + 128),
                  [f"wg{D - 128}_{c}", f"wu{D - 128}_{c}"] + ([f"d{r - 128}"] if r else []), down_proj))

  for r in range(0, tail0, DH):
    def out_proj(r=r):
      hq = r // DH
      lhs = jnp.broadcast_to(st["o", hq // REP][hq % REP:hq % REP + 1, :], (M, DH)).astype(bf16)
      accumulate("attn", jnp.dot(lhs, wo_v[pl.ds(r, DH), :], preferred_element_type=f32))
    tasks.append((f"o{r}", needs("wo", None, r, r + DH), [f"pv{r // DH // REP}_{n_kb - 1}"], out_proj))

  def last_head_as_column():
    a = st["o", HKV - 1][REP - 1:REP, :].astype(bf16).astype(f32)
    st["a_col"] = jnp.transpose(jnp.broadcast_to(a, (DH, DH)))
  tasks.append(("a_col", (0, 0), [f"pv{HKV - 1}_{n_kb - 1}"], last_head_as_column))

  x_copy = pltpu.make_async_copy(x_hbm, x_v, sem_small.at[0])
  wr_copy = pltpu.make_async_copy(wr_hbm, wr_v, sem_small.at[1])
  started, landed = [0, 0], [0, 0]
  for q, i in (e for events in periods for e in events):
    if started[q] < IN_FLIGHT[q]:
      copy(q, started[q]).start(priority=q)
      started[q] += 1
      if started == [0, 1]:
        x_copy.start()
        wr_copy.start()

  done = set()
  prelude = [layernorm_mean, layernorm_scale, router]

  def ready(limit):
    found, have = [], set(done)
    for task in tasks:
      name, need, after, _ = task
      if (name not in have and need[0] <= landed[0] and need[1] <= landed[1] and all(a in have for a in after)):
        found.append(task)
        have.add(name)
        if len(found) == limit:
          break
    return found

  def run(batch):
    for name, _, _, body in batch:
      body()
      done.add(name)

  tail_started = False
  for p, events in enumerate(periods):
    for q, i in events:
      copy(q, i).wait()
      landed[q] += 1
      if started[q] < len(streams[q]):
        copy(q, started[q]).start(priority=q)
        started[q] += 1
      elif q == 1 and not tail_started:
        tail_started = True
        for j in range(n_tail):
          tail_copy(j).start(priority=1)
    if LN_PERIOD <= p < LN_PERIOD + len(prelude):
      prelude[p - LN_PERIOD]()
    elif p >= LN_PERIOD + len(prelude):
      if p == len(periods) - 1:
        run(ready(len(tasks)))
      else:
        batch = ready(TASKS_PER_PERIOD)
        if len(batch) == TASKS_PER_PERIOD or p >= len(periods) - EAGER_PERIODS:
          run(batch)
  assert tail_started and len(done) == len(tasks)

  x, xn = st["x"], st["xn"]
  out = x + xn + (xn * 0.0 + st["y"][0:1] * st["r_sel"]) + st["attn"][0:1]
  part = None
  for j in range(n_tail):
    tail_copy(j).wait()
    w = wo_v[pl.ds(tail0 + j * TAIL_PIECE, TAIL_PIECE), :].astype(f32)
    a = st["a_col"][j * TAIL_PIECE:(j + 1) * TAIL_PIECE, :]
    prod = jnp.concatenate([w[:, c:c + DH] * a for c in range(0, D, DH)], axis=1)
    for s in range(0, TAIL_PIECE, 8):
      part = prod[s:s + 8] if part is None else part + prod[s:s + 8]
  out = out + jnp.sum(part, axis=0, keepdims=True)
  out_ref[...] = out.astype(bf16).reshape(1, 1, D)


@jax.jit
def pallas_parallel_sum__sliding_block_cached__moe_arch_mod__decode_kernel(
    A_x, A_k_cache, A_v_cache, A_wq, A_wo, B_x, B_w_r, B_w_gate, B_w_up, B_w_down,
):
  del B_x
  assert A_x.shape == (1, 1, D) and A_k_cache.shape[:2] == (1, HKV) and A_k_cache.shape[3] == DH
  window = min(4096, max(256, A_k_cache.shape[2] // 4))
  assert window % KEY_BLOCK == 0
  bf16 = jnp.bfloat16
  return pl.pallas_call(
      _kernel,
      in_specs=[pl.BlockSpec(memory_space=pl.ANY)] * 9,
      out_specs=pl.BlockSpec(memory_space=pltpu.VMEM),
      out_shape=jax.ShapeDtypeStruct((1, 1, D), bf16),
      scratch_shapes=[
          pltpu.VMEM((1, 1, D), bf16),
          pltpu.VMEM((D,), bf16),
          pltpu.VMEM((D, HQ * DH), bf16),
          pltpu.VMEM((HKV, window, DH), bf16),
          pltpu.VMEM((HKV, window, DH), bf16),
          pltpu.VMEM((HQ * DH, D), bf16),
          pltpu.VMEM((D, F), bf16),
          pltpu.VMEM((D, F), bf16),
          pltpu.VMEM((F, D), bf16),
          pltpu.SemaphoreType.DMA((IN_FLIGHT[0],)),
          pltpu.SemaphoreType.DMA((IN_FLIGHT[1],)),
          pltpu.SemaphoreType.DMA((2,)),
          pltpu.SemaphoreType.DMA((TAIL_ROWS // TAIL_PIECE,)),
      ],
      compiler_params=pltpu.CompilerParams(
          vmem_limit_bytes=64 * 1024 * 1024,
          disable_bounds_checks=True,
          disable_semaphore_checks=True,
      ),
      name="fused_decode",
  )(A_x, A_k_cache, A_v_cache, A_wq, A_wo, B_w_r, B_w_gate, B_w_up, B_w_down)
```
